```python
import os as _os
_os.environ.setdefault("JAX_PLATFORMS", "cpu")
import jax
import jax.numpy as jnp

def _softmax(x, axis=-1):
    return jax.nn.softmax(x, axis=axis)
def _gelu(x):
    return jax.nn.gelu(x, approximate=True)
def _silu(x):
    return jax.nn.silu(x)
def _sigmoid(x):
    return jax.nn.sigmoid(x)
def _layernorm(x, axis=-1, eps=1e-5):
    m = jnp.mean(x, axis=axis, keepdims=True)
    v = jnp.var(x, axis=axis, keepdims=True)
    return (x - m) / jnp.sqrt(v + eps)
def _scatter_add(tgt, idx, src, axis=0):
    return tgt.at[idx].add(src)
def _segment_sum(src, seg, n):
    return jax.ops.segment_sum(src, seg, n)
class _Rng:
    def __init__(self, key):
        self._k = key
    def _next(self):
        self._k, sub = jax.random.split(self._k)
        return sub
    def normal(self, shape):
        return jax.random.normal(self._next(), shape, dtype=jnp.bfloat16)
    def randint(self, lo, hi, shape):
        return jax.random.randint(self._next(), shape, lo, hi, dtype=jnp.int32)
    def uniform(self, shape, lo=0.0, hi=1.0):
        return jax.random.uniform(self._next(), shape, jnp.bfloat16, lo, hi)
    def permutation(self, n):
        return jax.random.permutation(self._next(), n)


kernel_name = 'concat_heads__gqa_block_cached__gqa_block_cached__near_ridge'

def setup_inputs():
    _rng = _Rng(jax.random.key(int.from_bytes(__import__("os").urandom(4), "little")))
    _w = (lambda a: (lambda t: t.astype(jnp.bfloat16) if jnp.issubdtype(t.dtype, jnp.floating) else t)(jnp.asarray(a)))
    def _A_setup():
        B, Sq, D = 16, 144, 448
        Hq, Hkv, Sk, Dh = 16, 8, 1024, 256
        assert Hq % Hkv == 0, (Hq, Hkv)
        return {
            "x": _w((lambda *s: _rng.normal(s) * 0.8)(B, Sq, D)),
            "k_cache": _w((lambda *s: _rng.normal(s) * 0.8)(B, Hkv, Sk, Dh)),
            "v_cache": _w((lambda *s: _rng.normal(s) * 0.05)(B, Hkv, Sk, Dh)),
            "wq": _w((lambda *s: _rng.normal(s) * 0.8)(D, Hq * Dh) * (D ** -0.5)),
            "wo": _w((lambda *s: _rng.normal(s) * 0.05)(Hq * Dh, D) * ((Hq * Dh) ** -0.5)),
        }
    _A_in = _A_setup()

    def _B_setup():
        B, Sq, D = 16, 144, 448
        Hq, Hkv, Sk, Dh = 16, 8, 1024, 256
        assert Hq % Hkv == 0, (Hq, Hkv)
        return {
            "x": _w((lambda *s: _rng.normal(s) * 0.8)(B, Sq, D)),
            "k_cache": _w((lambda *s: _rng.normal(s) * 0.8)(B, Hkv, Sk, Dh)),
            "v_cache": _w((lambda *s: _rng.normal(s) * 0.05)(B, Hkv, Sk, Dh)),
            "wq": _w((lambda *s: _rng.normal(s) * 0.8)(D, Hq * Dh) * (D ** -0.5)),
            "wo": _w((lambda *s: _rng.normal(s) * 0.05)(Hq * Dh, D) * ((Hq * Dh) ** -0.5)),
        }
    _B_in = _B_setup()

    return {
        "A_x": _A_in["x"],
        "A_k_cache": _A_in["k_cache"],
        "A_v_cache": _A_in["v_cache"],
        "A_wq": _A_in["wq"],
        "A_wo": _A_in["wo"],
        "B_x": _B_in["x"],
        "B_k_cache": _B_in["k_cache"],
        "B_v_cache": _B_in["v_cache"],
        "B_wq": _B_in["wq"],
        "B_wo": _B_in["wo"],
    }

def reference(A_x, A_k_cache, A_v_cache, A_wq, A_wo, B_x, B_k_cache, B_v_cache, B_wq, B_wo):
    def _A_ref(x, k_cache, v_cache, wq, wo):
        B, Sq, D = x.shape
        Hq, Dh = 16, 256
        Hkv = k_cache.shape[1]
        rep = Hq // Hkv
        q = (lambda x, *d: x.transpose(*d))((x @ wq).reshape(B, Sq, Hq, Dh), 0, 2, 1, 3)
        k = jnp.repeat(k_cache, rep, axis=1)
        v = jnp.repeat(v_cache, rep, axis=1)
        scores = jnp.einsum("bhqd,bhkd->bhqk", q, k) * (Dh ** -0.5)
        p = _softmax(scores, axis=-1)
        o = jnp.einsum("bhqk,bhkd->bhqd", p, v)
        return (lambda x, *d: x.transpose(*d))(o, 0, 2, 1, 3).reshape(B, Sq, Hq * Dh) @ wo

    def _B_ref(x, k_cache, v_cache, wq, wo):
        B, Sq, D = x.shape
        Hq, Dh = 16, 256
        Hkv = k_cache.shape[1]
        rep = Hq // Hkv
        q = (lambda x, *d: x.transpose(*d))((x @ wq).reshape(B, Sq, Hq, Dh), 0, 2, 1, 3)
        k = jnp.repeat(k_cache, rep, axis=1)
        v = jnp.repeat(v_cache, rep, axis=1)
        scores = jnp.einsum("bhqd,bhkd->bhqk", q, k) * (Dh ** -0.5)
        p = _softmax(scores, axis=-1)
        o = jnp.einsum("bhqk,bhkd->bhqd", p, v)
        return (lambda x, *d: x.transpose(*d))(o, 0, 2, 1, 3).reshape(B, Sq, Hq * Dh) @ wo

    a = _A_ref(A_x, A_k_cache, A_v_cache, A_wq, A_wo)
    b = _B_ref(B_x, B_k_cache, B_v_cache, B_wq, B_wo)
    return jnp.concatenate([a, b], axis=-1)
```

```python
import jax
import jax.numpy as jnp
import numpy as np
from jax import lax
import jax.experimental.pallas as pl
import jax.experimental.pallas.tpu as pltpu

B, SQ, D, HQ, HKV, SK, DH = 16, 144, 448, 16, 8, 1024, 256
REP = HQ // HKV
GW = REP * DH
M = REP * SQ
NTOK = B * SQ
ITEMS = HKV * B
LANES = 128
EXP2_SCALE = float(np.log2(np.e)) * DH ** -0.5

G = 12
PEEL = 4
NBLK = (2 * ITEMS - PEEL) // G
WEIGHT_STEP = 5
TB = 384
OUT_CUT = 768
NT = (((1,), (1,)), ((), ()))

assert NBLK * G + PEEL == 2 * ITEMS and G % 4 == 0 and PEEL % 4 == 0 and 3 * PEEL <= G
assert NBLK > HQ and G <= 2 * B


def _div(i, n):
    assert n & (n - 1) == 0
    return i >> (n.bit_length() - 1)


def _mod(i, n):
    assert n & (n - 1) == 0
    return i & (n - 1)


def _min(i, n):
    return min(i, n) if isinstance(i, int) else jnp.minimum(i, n)


def _ds(start, size, align):
    return pl.ds(start if isinstance(start, int) else pl.multiple_of(start, align), size)


def _start(copies):
    for c in copies:
        c.start()


def _wait(copies):
    for c in copies:
        c.wait()


def _kernel(xa, ka, va, wqa, woa, xb, kb, vb, wqb, wob, out_hbm,
            x_buf, k_buf, v_buf, wo_buf, o_buf, out_buf, s_buf, m_buf, q_buf, in_sem, out_sem):
    xs, ks, vs, wqs, wos = (xa, xb), (ka, kb), (va, vb), (wqa, wqb), (woa, wob)


    def first_item(i):
        return PEEL // 2 + i * (G // 2)

    def head_batch(i, u):
        pair = _min(PEEL // 4 + i * (G // 4) + u // 2, ITEMS // 2 - 1)
        return _div(pair, B // 2), _mod(pair, B // 2) * 2 + u % 2

    def is_first(i, j):
        return isinstance(i, int) and PEEL + i * G + j == 0

    def operand_copies(i, j, sems):
        slot, (u, br) = _mod(i, 2), divmod(j, 2)
        h, b = head_batch(i, u)
        x = [pltpu.make_async_copy(xs[br].at[b], x_buf.at[slot, j], sems[0])]
        k = [pltpu.make_async_copy(ks[br].at[b, h], k_buf.at[slot, j], sems[2])]
        if is_first(i, j):
            return x, [], k
        hp, bp = head_batch(i, (j - 1) // 2)
        return x, [pltpu.make_async_copy(vs[1 - br].at[bp, hp], v_buf.at[slot, j], sems[1])], k

    def wq_rows(h):
        return _ds(ITEMS * SQ + h * D, D, 16)

    def wq_copy(br, h, r, sem):
        src = wqs[br].at[:, _ds(_min(h, HKV - 1) * GW + r * DH, DH, DH)]
        return pltpu.make_async_copy(src, o_buf.at[br, wq_rows(h), _ds(r * DH, DH, DH)], sem)

    def weight_copies(i, sem):
        n = i + REP
        cps = [wq_copy(br, _div(_min(n, HQ), REP), _mod(n, REP), sem) for br in range(2)]
        for br in range(2):
            src = wos[br].at[:, _ds(_min(i, HQ - 1) * DH, DH, DH)]
            dst = wo_buf.at[br, _div(_min(i, HQ), REP), :, _ds(_mod(i, REP) * DH, DH, DH)]
            cps.append(pltpu.make_async_copy(src, dst, sem))
        return cps

    def step_copies(i, j):
        sem = in_sem.at[_mod(i, 2), j]
        return sum(operand_copies(i, j, [sem] * 3), []) + (weight_copies(i, sem) if j == WEIGHT_STEP else [])


    def queries(x_ref, h, br):
        x = x_ref[...]
        for r in range(REP):
            q = jnp.dot(x, o_buf[br, wq_rows(h), r * DH:(r + 1) * DH], preferred_element_type=jnp.float32)
            q_buf[r * SQ:(r + 1) * SQ, :] = (q * EXP2_SCALE).astype(q_buf.dtype)

    def row_max(s):
        m_buf[...] = jnp.broadcast_to(jnp.max(s, axis=-1, keepdims=True), (M, LANES))

    def scores(k_ref, with_max):
        s = lax.dot_general(q_buf[...], k_ref[...], NT, preferred_element_type=jnp.float32)
        s_buf[...] = s
        if with_max:
            row_max(s)

    def values(t, br, v_ref):
        acc = denom = None
        for c in range(0, SK, LANES):
            p = jnp.exp2(s_buf[:, c:c + LANES] - m_buf[...])
            denom = p if denom is None else denom + p
            o = jnp.dot(p.astype(v_ref.dtype), v_ref[c:c + LANES, :], preferred_element_type=jnp.float32)
            acc = o if acc is None else acc + o
        o = (acc * (1.0 / jnp.sum(denom, axis=-1, keepdims=True))).astype(o_buf.dtype)
        for r in range(REP):
            o_buf[br, _ds(t * SQ, SQ, 16), r * DH:(r + 1) * DH] = o[r * SQ:(r + 1) * SQ]

    def steps(i, js, sync):
        slot = _mod(i, 2)
        for j in js:
            u, br = divmod(j, 2)
            for stage in ((1, 0) if is_first(i, j - 1) else (0, 1)):
                sync(j, stage)
                if stage == 0:
                    queries(x_buf.at[slot, j], head_batch(i, u)[0], br)
                elif not is_first(i, j):
                    values(first_item(i) + (j - 1) // 2, 1 - br, v_buf.at[slot, j])
            sync(j, 2)
            scores(k_buf.at[slot, j], with_max=j != js[-1])

    def block(i, carry):
        def sync(j, stage):
            if stage == 0:
                _wait(step_copies(i, j))
                _start(step_copies(i + 1, j))

        row_max(s_buf[...])
        steps(i, range(G), sync)
        return carry


    lead = range(G - PEEL, G)
    head = {j: operand_copies(-1, j, [in_sem.at[1, 3 * (j - lead[0]) + n] for n in range(3)]) for j in lead}
    for br in range(2):
        head[lead[br]][0].extend(wq_copy(br, 0, r, in_sem.at[1, 3 * br]) for r in range(REP))
    for j in lead:
        _start(head[j][1] + head[j][0] + head[j][2])
    for j in range(G):
        _start(step_copies(0, j))
    steps(-1, lead, lambda j, stage: _wait(head[j][stage]))
    lax.fori_loop(0, NBLK, block, None)
    for j in range(G):
        _wait(step_copies(NBLK, j))
    row_max(s_buf[...])
    values(ITEMS - 1, 1, v_buf.at[NBLK % 2, 0])


    half = D % LANES
    main = D - half

    def out_copies(j):
        slot, edges = _mod(j, 2), (0, OUT_CUT, 2 * D)
        return {c1: pltpu.make_async_copy(out_buf.at[slot, :, c0:c1], out_hbm.at[_ds(j * TB, TB, TB), c0:c1],
                                          out_sem.at[slot])
                for c0, c1 in zip(edges, edges[1:])}

    def over_heads(f):
        acc = f(0)
        for h in range(1, HKV):
            acc = acc + f(h)
        return acc

    def project(j, carry):
        @pl.when(j >= 2)
        def _():
            _wait(out_copies(j - 2).values())

        out = out_buf.at[_mod(j, 2)]
        sends = out_copies(j)

        def o_rows(br, h):
            return o_buf[br, _ds(h * NTOK + j * TB, TB, 16), :]

        def seam():
            parts = [over_heads(lambda h: lax.dot_general(wo_buf[br, h, w0:w0 + half, :], o_rows(br, h), NT,
                                                          preferred_element_type=jnp.float32))
                     for br, w0 in ((0, main), (1, 0))]
            out[:, main:main + LANES] = jnp.concatenate(parts, axis=0).T.astype(out.dtype)

        for br, w0, c0 in ((0, 0, 0), (1, half, D + half)):
            for n in range(0, main, LANES):
                if (br, n) == (0, LANES):
                    seam()
                r = over_heads(lambda h: lax.dot_general(o_rows(br, h), wo_buf[br, h, w0 + n:w0 + n + LANES, :], NT,
                                                         preferred_element_type=jnp.float32))
                out[:, c0 + n:c0 + n + LANES] = r.astype(out.dtype)
                if c0 + n + LANES in sends:
                    sends[c0 + n + LANES].start()
        return carry

    n_out = NTOK // TB
    lax.fori_loop(0, n_out, project, None)
    _wait(out_copies(n_out - 2).values())
    _wait(out_copies(n_out - 1).values())


@jax.jit
def pallas_concat_heads__gqa_block_cached__gqa_block_cached__near_ridge_kernel(
    A_x: jax.Array,
    A_k_cache: jax.Array,
    A_v_cache: jax.Array,
    A_wq: jax.Array,
    A_wo: jax.Array,
    B_x: jax.Array,
    B_k_cache: jax.Array,
    B_v_cache: jax.Array,
    B_wq: jax.Array,
    B_wo: jax.Array,
):
    assert A_x.shape == B_x.shape == (B, SQ, D) and A_k_cache.shape == B_k_cache.shape == (B, HKV, SK, DH)
    dtype = A_x.dtype
    dma = pltpu.SemaphoreType.DMA
    out = pl.pallas_call(
        _kernel,
        in_specs=[pl.BlockSpec(memory_space=pltpu.HBM)] * 10,
        out_specs=pl.BlockSpec(memory_space=pltpu.HBM),
        out_shape=jax.ShapeDtypeStruct((NTOK, 2 * D), dtype),
        scratch_shapes=[
            pltpu.VMEM((2, G, SQ, D), dtype),
            pltpu.VMEM((2, G, SK, DH), dtype),
            pltpu.VMEM((2, G, SK, DH), dtype),
            pltpu.VMEM((2, HKV + 1, D, GW), dtype),
            pltpu.VMEM((2, ITEMS * SQ + (HKV + 1) * D, GW), dtype),
            pltpu.VMEM((2, TB, 2 * D), dtype),
            pltpu.VMEM((M, SK), jnp.float32),
            pltpu.VMEM((M, LANES), jnp.float32),
            pltpu.VMEM((M, DH), dtype),
            dma((2, G)),
            dma((2,)),
        ],
        compiler_params=pltpu.CompilerParams(
            vmem_limit_bytes=110 * 1024 * 1024,
            disable_bounds_checks=True,
            flags={"XLA_TPU_FORCE_LP_LLO_SCHEDULER": True, "XLA_TPU_RESCHEDULE_DMA_DONES": True},
        ),
    )(A_x, A_k_cache, A_v_cache, A_wq, A_wo.T, B_x, B_k_cache, B_v_cache, B_wq, B_wo.T)
    return out.reshape(B, SQ, 2 * D)
```

```python
import jax
import jax.numpy as jnp
import numpy as np
from jax import lax
import jax.experimental.pallas as pl
import jax.experimental.pallas.tpu as pltpu

B, SQ, D, HQ, HKV, SK, DH = 16, 144, 448, 16, 8, 1024, 256
REP = HQ // HKV
GW = REP * DH
M = REP * SQ
NTOK = B * SQ
ITEMS = HKV * B
LANES = 128
EXP2_SCALE = float(np.log2(np.e)) * DH ** -0.5

G = 12
PEEL = 4
NBLK = (2 * ITEMS - PEEL) // G
WEIGHT_STEP = 5
TB = 384
OUT_CUT = 768
NT = (((1,), (1,)), ((), ()))

assert NBLK * G + PEEL == 2 * ITEMS and G % 4 == 0 and PEEL % 4 == 0 and 3 * PEEL == G
assert NBLK > HQ and G <= 2 * B


def _div(i, n):
    assert n & (n - 1) == 0
    return i >> (n.bit_length() - 1)


def _mod(i, n):
    assert n & (n - 1) == 0
    return i & (n - 1)


def _min(i, n):
    return min(i, n) if isinstance(i, int) else jnp.minimum(i, n)


def _ds(start, size, align):
    return pl.ds(start if isinstance(start, int) else pl.multiple_of(start, align), size)


def _start(copies):
    for c in copies:
        c.start()


def _wait(copies):
    for c in copies:
        c.wait()


def _kernel(xa, ka, va, wqa, woa, xb, kb, vb, wqb, wob, out_hbm,
            x_buf, k_buf, v_buf, wo_buf, o_buf, out_buf, s_buf, m_buf, q_buf, in_sem, out_sem):
    xs, ks, vs, wqs, wos = (xa, xb), (ka, kb), (va, vb), (wqa, wqb), (woa, wob)


    def head_batch(i, u):
        pair = _min(PEEL // 4 + i * (G // 4) + u // 2, ITEMS // 2 - 1)
        return _div(pair, B // 2), _mod(pair, B // 2) * 2 + u % 2

    def is_first(i, j):
        return isinstance(i, int) and PEEL + i * G + j == 0

    def operand_copies(i, j, sems):
        slot, (u, br) = _mod(i, 2), divmod(j, 2)
        h, b = head_batch(i, u)
        x = [pltpu.make_async_copy(xs[br].at[b], x_buf.at[slot, j], sems[0])]
        k = [pltpu.make_async_copy(ks[br].at[b, h], k_buf.at[slot, j], sems[2])]
        if is_first(i, j):
            return x, [], k
        hp, bp = head_batch(i, (j - 1) // 2)
        return x, [pltpu.make_async_copy(vs[1 - br].at[bp, hp], v_buf.at[slot, j], sems[1])], k

    def wq_rows(h):
        return _ds(ITEMS * SQ + h * D, D, 16)

    def wq_copy(br, h, r, sem):
        src = wqs[br].at[:, _ds(_min(h, HKV - 1) * GW + r * DH, DH, DH)]
        return pltpu.make_async_copy(src, o_buf.at[br, wq_rows(h), _ds(r * DH, DH, DH)], sem)

    def weight_copies(i, sem):
        n = i + REP
        cps = [wq_copy(br, _div(_min(n, HQ), REP), _mod(n, REP), sem) for br in range(2)]
        for br in range(2):
            src = wos[br].at[:, _ds(_min(i, HQ - 1) * DH, DH, DH)]
            dst = wo_buf.at[br, _div(_min(i, HQ), REP), :, _ds(_mod(i, REP) * DH, DH, DH)]
            cps.append(pltpu.make_async_copy(src, dst, sem))
        return cps

    def step_copies(i, j):
        sem = in_sem.at[_mod(i, 2), j]
        return sum(operand_copies(i, j, [sem] * 3), []) + (weight_copies(i, sem) if j == WEIGHT_STEP else [])


    def queries(x_ref, h, br):
        x = x_ref[...]
        for r in range(REP):
            q = jnp.dot(x, o_buf[br, wq_rows(h), r * DH:(r + 1) * DH], preferred_element_type=jnp.float32)
            q_buf[r * SQ:(r + 1) * SQ, :] = q.astype(q_buf.dtype)

    def row_max(s):
        m_buf[...] = jnp.broadcast_to(jnp.max(s, axis=-1, keepdims=True), (M, LANES))

    def scores(k_ref, finish_max):
        s = lax.dot_general(q_buf[...], k_ref[...], NT, preferred_element_type=jnp.float32)
        s_buf[...] = s
        if finish_max:
            row_max(s)
        else:
            m = s[:, :LANES]
            for c in range(LANES, SK, LANES):
                m = jnp.maximum(m, s[:, c:c + LANES])
            m_buf[...] = m

    def values(row, br, v_ref):
        acc = denom = None
        for c in range(0, SK, LANES):
            p = jnp.exp2((s_buf[:, c:c + LANES] - m_buf[...]) * EXP2_SCALE)
            denom = p if denom is None else denom + p
            o = jnp.dot(p.astype(v_ref.dtype), v_ref[c:c + LANES, :], preferred_element_type=jnp.float32)
            acc = o if acc is None else acc + o
        o = (acc * (1.0 / jnp.sum(denom, axis=-1, keepdims=True))).astype(o_buf.dtype)
        for r in range(REP):
            o_buf[br, _ds(row, SQ, 16), r * DH:(r + 1) * DH] = o[r * SQ:(r + 1) * SQ]

    def steps(i, js, sync):
        slot, first_row = _mod(i, 2), PEEL // 2 * SQ + i * (G // 2 * SQ)
        for j in js:
            u, br = divmod(j, 2)
            for stage in ((1, 0) if is_first(i, j - 1) else (0, 1)):
                sync(j, stage)
                if stage == 0:
                    queries(x_buf.at[slot, j], head_batch(i, u)[0], br)
                elif not is_first(i, j):
                    values(first_row + (j - 1) // 2 * SQ, 1 - br, v_buf.at[slot, j])
            sync(j, 2)
            scores(k_buf.at[slot, j], finish_max=j != js[-1])

    def block(i, carry):
        def sync(j, stage):
            if stage == 0:
                _wait(step_copies(i, j))
                _start(step_copies(i + 1, j))

        row_max(m_buf[...])
        steps(i, range(G), sync)
        return carry


    lead = range(G - PEEL, G)
    head = {j: operand_copies(-1, j, [in_sem.at[1, 3 * (j - lead[0]) + n] for n in range(3)]) for j in lead}
    for br in range(2):
        head[lead[br]][0].extend(wq_copy(br, 0, r, in_sem.at[1, 3 * br]) for r in range(REP))
    for j in lead:
        _start(head[j][1] + head[j][0] + head[j][2])

    def lead_sync(j, stage):
        _wait(head[j][stage])
        _start(step_copies(0, 3 * (j - lead[0]) + stage))

    steps(-1, lead, lead_sync)
    lax.fori_loop(0, NBLK, block, None)
    for j in range(G):
        _wait(step_copies(NBLK, j))
    row_max(m_buf[...])
    values((ITEMS - 1) * SQ, 1, v_buf.at[NBLK % 2, 0])


    half = D % LANES
    main = D - half

    def out_copies(j):
        slot, edges = _mod(j, 2), (0, OUT_CUT, 2 * D)
        return {c1: pltpu.make_async_copy(out_buf.at[slot, :, c0:c1], out_hbm.at[_ds(j * TB, TB, TB), c0:c1],
                                          out_sem.at[slot])
                for c0, c1 in zip(edges, edges[1:])}

    def over_heads(f):
        acc = f(0)
        for h in range(1, HKV):
            acc = acc + f(h)
        return acc

    def project(j, carry):
        @pl.when(j >= 2)
        def _():
            _wait(out_copies(j - 2).values())

        out = out_buf.at[_mod(j, 2)]
        sends = out_copies(j)

        def o_rows(br, h):
            return o_buf[br, _ds(h * NTOK + j * TB, TB, 16), :]

        def seam():
            parts = [over_heads(lambda h: lax.dot_general(wo_buf[br, h, w0:w0 + half, :], o_rows(br, h), NT,
                                                          preferred_element_type=jnp.float32))
                     for br, w0 in ((0, main), (1, 0))]
            out[:, main:main + LANES] = jnp.concatenate(parts, axis=0).T.astype(out.dtype)

        for br, w0, c0 in ((0, 0, 0), (1, half, D + half)):
            for n in range(0, main, LANES):
                if (br, n) == (0, LANES):
                    seam()
                r = over_heads(lambda h: lax.dot_general(o_rows(br, h), wo_buf[br, h, w0 + n:w0 + n + LANES, :], NT,
                                                         preferred_element_type=jnp.float32))
                out[:, c0 + n:c0 + n + LANES] = r.astype(out.dtype)
                if c0 + n + LANES in sends:
                    sends[c0 + n + LANES].start()
        return carry

    n_out = NTOK // TB
    lax.fori_loop(0, n_out, project, None)
    _wait(out_copies(n_out - 2).values())
    _wait(out_copies(n_out - 1).values())


@jax.jit
def pallas_concat_heads__gqa_block_cached__gqa_block_cached__near_ridge_kernel(
    A_x: jax.Array,
    A_k_cache: jax.Array,
    A_v_cache: jax.Array,
    A_wq: jax.Array,
    A_wo: jax.Array,
    B_x: jax.Array,
    B_k_cache: jax.Array,
    B_v_cache: jax.Array,
    B_wq: jax.Array,
    B_wo: jax.Array,
):
    assert A_x.shape == B_x.shape == (B, SQ, D) and A_k_cache.shape == B_k_cache.shape == (B, HKV, SK, DH)
    dtype = A_x.dtype
    dma = pltpu.SemaphoreType.DMA
    out = pl.pallas_call(
        _kernel,
        in_specs=[pl.BlockSpec(memory_space=pltpu.HBM)] * 10,
        out_specs=pl.BlockSpec(memory_space=pltpu.HBM),
        out_shape=jax.ShapeDtypeStruct((NTOK, 2 * D), dtype),
        scratch_shapes=[
            pltpu.VMEM((2, G, SQ, D), dtype),
            pltpu.VMEM((2, G, SK, DH), dtype),
            pltpu.VMEM((2, G, SK, DH), dtype),
            pltpu.VMEM((2, HKV + 1, D, GW), dtype),
            pltpu.VMEM((2, ITEMS * SQ + (HKV + 1) * D, GW), dtype),
            pltpu.VMEM((2, TB, 2 * D), dtype),
            pltpu.VMEM((M, SK), jnp.float32),
            pltpu.VMEM((M, LANES), jnp.float32),
            pltpu.VMEM((M, DH), dtype),
            dma((2, G)),
            dma((2,)),
        ],
        compiler_params=pltpu.CompilerParams(
            vmem_limit_bytes=110 * 1024 * 1024,
            disable_bounds_checks=True,
            flags={"XLA_TPU_FORCE_LP_LLO_SCHEDULER": True, "XLA_TPU_RESCHEDULE_DMA_DONES": True},
        ),
    )(A_x, A_k_cache, A_v_cache, A_wq, A_wo.T, B_x, B_k_cache, B_v_cache, B_wq, B_wo.T)
    return out.reshape(B, SQ, 2 * D)
```
